```python
import jax
import jax.numpy as jnp

def _softmax(x, axis=-1):
    return jax.nn.softmax(x, axis=axis)

def _gelu(x):
    return jax.nn.gelu(x, approximate=True)

def _silu(x):
    return jax.nn.silu(x)

def _sigmoid(x):
    return jax.nn.sigmoid(x)

def _layernorm(x, axis=-1, eps=1e-05):
    m = jnp.mean(x, axis=axis, keepdims=True)
    v = jnp.var(x, axis=axis, keepdims=True)
    return (x - m) / jnp.sqrt(v + eps)

def _scatter_add(tgt, idx, src, axis=0):
    return tgt.at[idx].add(src)

def _segment_sum(src, seg, n):
    return jax.ops.segment_sum(src, seg, n)

class _Rng:

    def __init__(self, key):
        self._k = key

    def _next(self):
        self._k, sub = jax.random.split(self._k)
        return sub

    def normal(self, shape):
        return jax.random.normal(self._next(), shape, dtype=jnp.bfloat16)

    def randint(self, lo, hi, shape):
        return jax.random.randint(self._next(), shape, lo, hi, dtype=jnp.int32)

    def uniform(self, shape, lo=0.0, hi=1.0):
        return jax.random.uniform(self._next(), shape, jnp.bfloat16, lo, hi)

    def permutation(self, n):
        return jax.random.permutation(self._next(), n)
kernel_name = 'adaLN_cond__sliding_local_dilated__mixer_s_mlp__prompt'

def setup_inputs():
    _rng = _Rng(jax.random.key(int.from_bytes(__import__("os").urandom(4), "little")))
    _w = lambda a: (lambda t: t.astype(jnp.bfloat16) if jnp.issubdtype(t.dtype, jnp.floating) else t)(jnp.asarray(a))

    def _A_setup():
        B, S, D = (1, 2048, 1024)
        return {'x': _w((lambda *s: _rng.normal(s) * 0.05)(B, S, D)), 'wqkv': _w((lambda *s: _rng.normal(s) * 0.05)(D, 3 * D)), 'wo': _w((lambda *s: _rng.normal(s) * 0.05)(D, D))}
    _A_in = _A_setup()

    def _B_setup():
        B, S, D, F = (1, 2048, 1024, 3584)
        return {'x': _w((lambda *s: _rng.normal(s) * 0.05)(B, S, D)), 'w1': _w((lambda *s: _rng.normal(s) * 0.05)(D, D) * D ** (-0.5)), 'w2': _w((lambda *s: _rng.normal(s) * 0.05)(D, D) * D ** (-0.5)), 'w3': _w((lambda *s: _rng.normal(s) * 0.05)(D, F) * D ** (-0.5)), 'w4': _w((lambda *s: _rng.normal(s) * 0.05)(F, D) * F ** (-0.5))}
    _B_in = _B_setup()
    return {'A_x': _A_in['x'], 'A_wqkv': _A_in['wqkv'], 'A_wo': _A_in['wo'], 'B_x': _B_in['x'], 'B_w1': _B_in['w1'], 'B_w2': _B_in['w2'], 'B_w3': _B_in['w3'], 'B_w4': _B_in['w4'], 'c': _w((lambda *s: _rng.normal(s) * 0.05)(1, 1024)), 'w_mod': _w((lambda *s: _rng.normal(s) * 0.05)(1024, 6 * 1024) * 1024 ** (-0.5))}

def reference(A_x, A_wqkv, A_wo, B_x, B_w1, B_w2, B_w3, B_w4, c, w_mod):

    def _A_ref(x, wqkv, wo):
        B, S, D = x.shape
        H = 32
        Dh = D // H
        W, dil = (8, 2)
        qkv = (lambda x, *d: x.transpose(*d))((x @ wqkv).reshape(B, S, 3, H, Dh), 2, 0, 3, 1, 4)
        q, k, v = (qkv[0], qkv[1], qkv[2])
        scale = Dh ** (-0.5)
        pos = jnp.arange(S)
        off = jnp.arange(W) * dil
        idx = pos[:, None] - off[None, :]
        mask = idx >= 0
        idx_c = jnp.where(mask, idx, 0).reshape(-1)
        kg = k[:, :, idx_c, :].reshape(B, H, S, W, Dh)
        vg = v[:, :, idx_c, :].reshape(B, H, S, W, Dh)
        logits = jnp.einsum('bhsd,bhswd->bhsw', q, kg) * scale
        logits = jnp.where(mask[None, None, :, :], logits, -1000000000.0)
        attn = _softmax(logits, axis=-1)
        o = jnp.einsum('bhsw,bhswd->bhsd', attn, vg)
        return (lambda x, *d: x.transpose(*d))(o, 0, 2, 1, 3).reshape(B, S, D) @ wo

    def _B_ref(x, w1, w2, w3, w4):
        B, S, D = x.shape
        h = _gelu(_layernorm(x, axis=-1) @ w1)
        c = D // 4
        g0 = jnp.pad(h[:, :, 0 * c:1 * c], ((0, 0), (1, 0), (0, 0)))[:, :S, :]
        g1 = jnp.pad(h[:, :, 1 * c:2 * c], ((0, 0), (0, 1), (0, 0)))[:, 1:, :]
        g2 = jnp.pad(h[:, :, 2 * c:3 * c], ((0, 0), (2, 0), (0, 0)))[:, :S, :]
        g3 = jnp.pad(h[:, :, 3 * c:], ((0, 0), (0, 2), (0, 0)))[:, 2:, :]
        hs = jnp.concatenate([g0, g1, g2, g3], axis=-1) @ w2
        x1 = x + hs
        h2 = _gelu(_layernorm(x1, axis=-1) @ w3) @ w4
        return x1 + h2
    x = A_x
    mod = (_silu(c) @ w_mod).reshape(c.shape[0], 6, 1, -1)
    sa, ca, ga, sb, cb, gb = (mod[:, 0].copy(), mod[:, 1].copy(), mod[:, 2].copy(), mod[:, 3].copy(), mod[:, 4].copy(), mod[:, 5].copy())
    h = _layernorm(x, axis=-1) * (1 + ca) + sa
    x = x + ga * _A_ref(h, A_wqkv, A_wo)
    h = _layernorm(x, axis=-1) * (1 + cb) + sb
    x = x + gb * _B_ref(h, B_w1, B_w2, B_w3, B_w4)
    return x
```

```python
import functools

import jax
import jax.numpy as jnp
import numpy as np
import jax.experimental.pallas as pl
import jax.experimental.pallas.tpu as pltpu

H = 32
W = 8
DIL = 2
HALO = 16
PAD = 8
EPS = 1e-05
LAG = 1
T = 256

_F32 = jnp.float32
_BF16 = jnp.bfloat16


def _ln(x):
    m = jnp.mean(x, axis=-1, keepdims=True)
    d = x - m
    v = jnp.mean(d * d, axis=-1, keepdims=True)
    return d * jax.lax.rsqrt(v + EPS)


def _gelu(x):
    c0 = float(np.sqrt(2.0 / np.pi))
    c1 = float(np.sqrt(2.0 / np.pi) * 0.044715)
    u = x * (c0 + c1 * (x * x))
    return (0.5 * x) * (1.0 + jnp.tanh(u))


def _dot(a, b):
    return jnp.dot(a, b, preferred_element_type=_F32)


def _swap_bits(vs):
    lane = jax.lax.broadcasted_iota(jnp.int32, vs[0].shape, 1)
    for k in range(3):
        s = 4 << k
        hi = (lane & s) != 0
        nv = list(vs)
        for a in range(8):
            if a & (1 << k):
                continue
            b = a | (1 << k)
            nv[a] = jnp.where(hi, pltpu.roll(vs[b], s, 1), vs[a])
            nv[b] = jnp.where(hi, vs[b], pltpu.roll(vs[a], 128 - s, 1))
        vs = nv
    return vs


def _kernel(x_ref, c_ref, wqkv_h, wo_h, w1_h, w2_h, w3_h, w4_h, wmod_h,
            o_ref,
            wqkv, wo, w1, w2, w3, w4, wmod, mod, k_s, v_s, xa_s, hb_s, h1_s, sems,
            *, S, D, F):
    i = pl.program_id(0)
    nT = S // T
    Dh = D // H
    G = D // 128
    NQ = 4
    RQ = D // NQ

    def mod_copy(j):
        return pltpu.make_async_copy(wmod_h.at[:, pl.ds(j * 2 * D, 2 * D)],
                                     wmod.at[:, pl.ds(j * 2 * D, 2 * D)], sems.at[j])

    def qkv_copy(j):
        return pltpu.make_async_copy(wqkv_h.at[pl.ds(j * RQ, RQ)],
                                     wqkv.at[pl.ds(j * RQ, RQ)], sems.at[8 + j])
    cp_o = pltpu.make_async_copy(wo_h, wo, sems.at[3])
    cp_1 = pltpu.make_async_copy(w1_h, w1, sems.at[4])
    cp_2 = pltpu.make_async_copy(w2_h, w2, sems.at[5])
    cp_3 = pltpu.make_async_copy(w3_h, w3, sems.at[6])
    cp_4 = pltpu.make_async_copy(w4_h, w4, sems.at[7])

    def mrow(j):
        return mod[0:1, j * D:(j + 1) * D]

    def mod_chunk(j):
        cc = c_ref[...].astype(_F32)
        sc = (cc * jax.nn.sigmoid(cc)).astype(_BF16)
        sc = jnp.broadcast_to(sc, (16, D))
        mod_copy(j).wait()
        mod[:, j * 2 * D:(j + 1) * 2 * D] = _dot(sc, wmod[:, j * 2 * D:(j + 1) * 2 * D])

    @pl.when(i == 0)
    def _():
        mod_copy(0).start()
        for j in range(NQ):
            qkv_copy(j).start()
        cp_o.start()
        mod_copy(1).start()
        mod_copy(2).start()
        cp_1.start()
        cp_2.start()
        cp_3.start()
        cp_4.start()
        k_s[:, 0:HALO, :] = jnp.zeros((G, HALO, 128), _F32)
        v_s[:, 0:HALO, :] = jnp.zeros((G, HALO, 128), _F32)
        h1_s[0:PAD, :] = jnp.zeros((PAD, D), _F32)
        h1_s[PAD + S:PAD + S + PAD, :] = jnp.zeros((PAD, D), _F32)
        mod_chunk(0)

        def perm(t, _):
            for j in range(NQ):
                @pl.when(t == j * (RQ // 64))
                def _():
                    qkv_copy(j).wait()
            rows = pl.ds(pl.multiple_of(t * 64, 64), 64)
            for p in range(3):
                vs = [pltpu.bitcast(wqkv[rows, p * D + g * 128:p * D + (g + 1) * 128], jnp.int32)
                      for g in range(G)]
                vs = _swap_bits(vs)
                for g in range(G):
                    wqkv[rows, p * D + g * 128:p * D + (g + 1) * 128] = pltpu.bitcast(vs[g], _BF16)
        jax.lax.fori_loop(0, D // 64, perm, None)

    @pl.when(i < nT)
    def _():
        x = x_ref[...].astype(_F32)
        h = (_ln(x) * (1.0 + mrow(1)) + mrow(0)).astype(_BF16)
        q = _dot(h, wqkv[:, 0:D]) * (Dh ** -0.5)
        k = _dot(h, wqkv[:, D:2 * D])
        v = _dot(h, wqkv[:, 2 * D:3 * D])
        for g in range(G):
            k_s[g, HALO:HALO + T, :] = k[:, g * 128:(g + 1) * 128]
            v_s[g, HALO:HALO + T, :] = v[:, g * 128:(g + 1) * 128]
        r = jax.lax.broadcasted_iota(jnp.int32, (128, 128), 0) >> 2
        cidx = jax.lax.broadcasted_iota(jnp.int32, (128, 128), 1) >> 2
        bd = (r == cidx).astype(_BF16)
        pos = i * T + jax.lax.broadcasted_iota(jnp.int32, (T, 128), 0)
        parts = []
        for w in range(W):
            lo = HALO - DIL * w
            s = functools.reduce(jnp.add, [q[:, g * 128:(g + 1) * 128] * k_s[g, lo:lo + T, :]
                                           for g in range(G)])
            parts.append(s.astype(_BF16))
        lgs = _dot(jnp.concatenate(parts, axis=0), bd)
        lg = [lgs[w * T:(w + 1) * T] for w in range(W)]
        lg = [s if w == 0 else jnp.where(pos >= DIL * w, s, -1e9) for w, s in enumerate(lg)]
        m = functools.reduce(jnp.maximum, lg)
        ps = [jnp.exp(s - m) for s in lg]
        inv = 1.0 / functools.reduce(jnp.add, ps)
        ps = [p * inv for p in ps]
        outs = []
        for g in range(G):
            acc = functools.reduce(jnp.add, [ps[w] * v_s[g, HALO - DIL * w:HALO - DIL * w + T, :]
                                             for w in range(W)])
            outs.append(acc.astype(_BF16))
        o = jnp.concatenate(outs, axis=-1)
        k_s[:, 0:HALO, :] = k_s[:, T:T + HALO, :]
        v_s[:, 0:HALO, :] = v_s[:, T:T + HALO, :]

        @pl.when(i == 0)
        def _():
            cp_o.wait()
            for ct in range(G):
                cs = slice(ct * 128, (ct + 1) * 128)
                w32 = pltpu.bitcast(wo[:, cs], jnp.int32)
                for g in range(G):
                    pieces = []
                    for l in range(H):
                        hh = (l & 7) * 4 + (l >> 3)
                        r0 = hh * (Dh // 2) + g * 2
                        pieces.append(w32[r0:r0 + 2])
                    wo[g * 128:(g + 1) * 128, cs] = pltpu.bitcast(jnp.concatenate(pieces, axis=0), _BF16)
            mod_chunk(1)
            mod_chunk(2)
            cp_1.wait()

        xa = x_ref[...].astype(_F32) + mrow(2) * _dot(o, wo[...])
        slot = i % (LAG + 1)
        xa_s[slot] = xa
        hb = _ln(xa) * (1.0 + mrow(4)) + mrow(3)
        hb_s[slot] = hb
        h1 = _gelu(_dot(_ln(hb).astype(_BF16), w1[...]))
        h1_s[pl.ds(pl.multiple_of(PAD + i * T, 8), T), :] = h1

    @pl.when(i == LAG)
    def _():
        cp_2.wait()
        cp_3.wait()
        cp_4.wait()

    @pl.when(i >= LAG)
    def _():
        j = i - LAG
        slot = j % (LAG + 1)
        c4 = D // 4
        base = pl.multiple_of(j * T, 8)
        win = h1_s[pl.ds(base, T + 2 * PAD), :]
        g0 = win[PAD - 1:PAD - 1 + T, 0:c4]
        g1 = win[PAD + 1:PAD + 1 + T, c4:2 * c4]
        g2 = win[PAD - 2:PAD - 2 + T, 2 * c4:3 * c4]
        g3 = win[PAD + 2:PAD + 2 + T, 3 * c4:]
        gs = jnp.concatenate([g0, g1, g2, g3], axis=-1).astype(_BF16)
        x1 = hb_s[slot] + _dot(gs, w2[...])
        n1 = _ln(x1).astype(_BF16)
        h2 = None
        FC = 512
        for f in range(F // FC):
            t = _gelu(_dot(n1, w3[:, f * FC:(f + 1) * FC])).astype(_BF16)
            t = _dot(t, w4[f * FC:(f + 1) * FC, :])
            h2 = t if h2 is None else h2 + t
        o_ref[...] = (xa_s[slot] + mrow(5) * (x1 + h2)).astype(o_ref.dtype)


@jax.jit
def pallas_adaLN_cond__sliding_local_dilated__mixer_s_mlp__prompt_kernel(
    A_x: jax.Array,
    A_wqkv: jax.Array,
    A_wo: jax.Array,
    B_x: jax.Array,
    B_w1: jax.Array,
    B_w2: jax.Array,
    B_w3: jax.Array,
    B_w4: jax.Array,
    c: jax.Array,
    w_mod: jax.Array,
):
    del B_x
    B, S, D = A_x.shape
    F = B_w3.shape[1]
    assert B == 1 and S % T == 0
    nT = S // T
    x2 = A_x.reshape(S, D)
    hbm = pl.BlockSpec(memory_space=pl.ANY)
    out = pl.pallas_call(
        functools.partial(_kernel, S=S, D=D, F=F),
        grid=(nT + LAG,),
        in_specs=[
            pl.BlockSpec((T, D), lambda i: (jnp.minimum(i, nT - 1), 0)),
            pl.BlockSpec((1, D), lambda i: (0, 0)),
            hbm, hbm, hbm, hbm, hbm, hbm, hbm,
        ],
        out_specs=pl.BlockSpec((T, D), lambda i: (jnp.maximum(i - LAG, 0), 0)),
        out_shape=jax.ShapeDtypeStruct((S, D), A_x.dtype),
        scratch_shapes=[
            pltpu.VMEM((D, 3 * D), _BF16),
            pltpu.VMEM((D, D), _BF16),
            pltpu.VMEM((D, D), _BF16),
            pltpu.VMEM((D, D), _BF16),
            pltpu.VMEM((D, F), _BF16),
            pltpu.VMEM((F, D), _BF16),
            pltpu.VMEM((D, 6 * D), _BF16),
            pltpu.VMEM((16, 6 * D), _F32),
            pltpu.VMEM((D // 128, HALO + T, 128), _F32),
            pltpu.VMEM((D // 128, HALO + T, 128), _F32),
            pltpu.VMEM((LAG + 1, T, D), _F32),
            pltpu.VMEM((LAG + 1, T, D), _F32),
            pltpu.VMEM((S + 2 * PAD, D), _F32),
            pltpu.SemaphoreType.DMA((12,)),
        ],
        compiler_params=pltpu.CompilerParams(
            dimension_semantics=("arbitrary",),
            vmem_limit_bytes=100 * 1024 * 1024,
        ),
    )(x2, c, A_wqkv, A_wo, B_w1, B_w2, B_w3, B_w4, w_mod)
    return out.reshape(B, S, D)
```

```python
import functools

import jax
import jax.numpy as jnp
import numpy as np
import jax.experimental.pallas as pl
import jax.experimental.pallas.tpu as pltpu

H = 32
W = 8
DIL = 2
HALO = 16
PAD = 8
EPS = 1e-05
LAG = 1
NH = 2
MODC = (0, 2, 5, 6)
T = 256

_F32 = jnp.float32
_BF16 = jnp.bfloat16


def _ln(x):
    m = jnp.mean(x, axis=-1, keepdims=True)
    d = x - m
    v = jnp.mean(d * d, axis=-1, keepdims=True)
    return d * jax.lax.rsqrt(v + EPS)


def _gelu(x):
    c0 = float(np.sqrt(2.0 / np.pi))
    c1 = float(np.sqrt(2.0 / np.pi) * 0.044715)
    u = x * (c0 + c1 * (x * x))
    return (0.5 * x) * (1.0 + jnp.tanh(u))


def _dot(a, b):
    return jnp.dot(a, b, preferred_element_type=_F32)


def _swap_bits(vs):
    lane = jax.lax.broadcasted_iota(jnp.int32, vs[0].shape, 1)
    for k in range(3):
        s = 4 << k
        hi = (lane & s) != 0
        nv = list(vs)
        for a in range(8):
            if a & (1 << k):
                continue
            b = a | (1 << k)
            nv[a] = jnp.where(hi, pltpu.roll(vs[b], s, 1), vs[a])
            nv[b] = jnp.where(hi, vs[b], pltpu.roll(vs[a], 128 - s, 1))
        vs = nv
    return vs


def _kernel(x_ref, c_ref, wqkv_h, wo_h, w1_h, w2_h, w3_h, w4_h, wmod_h,
            o_ref,
            wqkv, wo, w1, w2, w3, w4, wmod, mod, k_s, v_s, xa_s, hb_s, h1_s, sems,
            *, S, D, F):
    i = pl.program_id(0)
    nT = S // T
    Dh = D // H
    G = D // 128
    NQ = 4
    RQ = D // NQ

    def mod_copy(j):
        return pltpu.make_async_copy(wmod_h.at[:, pl.ds(MODC[j] * D, (MODC[j + 1] - MODC[j]) * D)],
                                     wmod.at[:, pl.ds(MODC[j] * D, (MODC[j + 1] - MODC[j]) * D)], sems.at[j])

    def qkv_copy(j):
        return pltpu.make_async_copy(wqkv_h.at[pl.ds(j * RQ, RQ)],
                                     wqkv.at[pl.ds(j * RQ, RQ)], sems.at[8 + j])
    cp_o = pltpu.make_async_copy(wo_h, wo, sems.at[3])
    cp_1 = pltpu.make_async_copy(w1_h, w1, sems.at[4])
    cp_2 = pltpu.make_async_copy(w2_h, w2, sems.at[5])
    cp_3 = pltpu.make_async_copy(w3_h, w3, sems.at[6])
    cp_4 = pltpu.make_async_copy(w4_h, w4, sems.at[7])

    def mrow(j):
        return mod[0:1, j * D:(j + 1) * D]

    def mod_chunk(j):
        cc = c_ref[...].astype(_F32)
        sc = (cc * jax.nn.sigmoid(cc)).astype(_BF16)
        sc = jnp.broadcast_to(sc, (16, D))
        mod_copy(j).wait()
        mod[:, MODC[j] * D:MODC[j + 1] * D] = _dot(sc, wmod[:, MODC[j] * D:MODC[j + 1] * D])

    @pl.when(i == 0)
    def _():
        mod_copy(0).start()
        for j in range(NQ):
            qkv_copy(j).start()
        cp_o.start()
        mod_copy(1).start()
        cp_1.start()
        mod_copy(2).start()
        cp_2.start()
        cp_3.start()
        cp_4.start()
        k_s[:, 0:HALO, :] = jnp.zeros((G, HALO, 128), _F32)
        v_s[:, 0:HALO, :] = jnp.zeros((G, HALO, 128), _F32)
        h1_s[0:PAD, :] = jnp.zeros((PAD, D), _F32)
        h1_s[PAD + S:PAD + S + PAD, :] = jnp.zeros((PAD, D), _F32)
        mod_chunk(0)

        def perm(t, _):
            for j in range(NQ):
                @pl.when(t == j * (RQ // 64))
                def _():
                    qkv_copy(j).wait()
            rows = pl.ds(pl.multiple_of(t * 64, 64), 64)
            for p in range(3):
                vs = [pltpu.bitcast(wqkv[rows, p * D + g * 128:p * D + (g + 1) * 128], jnp.int32)
                      for g in range(G)]
                vs = _swap_bits(vs)
                for g in range(G):
                    wqkv[rows, p * D + g * 128:p * D + (g + 1) * 128] = pltpu.bitcast(vs[g], _BF16)
        jax.lax.fori_loop(0, D // 64, perm, None)

    R = T // NH

    @pl.when(i < nT)
    def _():
        slot = i % (LAG + 1)

        def ln1(u):
            x = x_ref[u * R:(u + 1) * R, :].astype(_F32)
            return (_ln(x) * (1.0 + mrow(1)) + mrow(0)).astype(_BF16)

        def qkv(u, h):
            lo = HALO + u * R
            k = _dot(h, wqkv[:, D:2 * D])
            for g in range(G):
                k_s[g, lo:lo + R, :] = k[:, g * 128:(g + 1) * 128]
            q = _dot(h, wqkv[:, 0:D]) * (Dh ** -0.5)
            v = _dot(h, wqkv[:, 2 * D:3 * D])
            for g in range(G):
                v_s[g, lo:lo + R, :] = v[:, g * 128:(g + 1) * 128]
            return q

        def attn(u, q):
            r = jax.lax.broadcasted_iota(jnp.int32, (128, 128), 0) >> 2
            cidx = jax.lax.broadcasted_iota(jnp.int32, (128, 128), 1) >> 2
            bd = (r == cidx).astype(_BF16)
            pos = i * T + u * R + jax.lax.broadcasted_iota(jnp.int32, (R, 128), 0)
            los = [HALO + u * R - DIL * w for w in range(W)]
            parts = []
            for lo in los:
                s = functools.reduce(jnp.add, [q[:, g * 128:(g + 1) * 128] * k_s[g, lo:lo + R, :]
                                               for g in range(G)])
                parts.append(s.astype(_BF16))
            lgs = _dot(jnp.concatenate(parts, axis=0), bd)
            lg = [lgs[w * R:(w + 1) * R] for w in range(W)]
            lg = [s if (w == 0 or u > 0) else jnp.where(pos >= DIL * w, s, -1e9) for w, s in enumerate(lg)]
            m = functools.reduce(jnp.maximum, lg)
            ps = [jnp.exp(s - m) for s in lg]
            inv = 1.0 / functools.reduce(jnp.add, ps)
            ps = [p * inv for p in ps]
            outs = []
            for g in range(G):
                acc = functools.reduce(jnp.add, [ps[w] * v_s[g, lo:lo + R, :]
                                                 for w, lo in enumerate(los)])
                outs.append(acc.astype(_BF16))
            return jnp.concatenate(outs, axis=-1)

        def ln23(u, a):
            rs = slice(u * R, (u + 1) * R)
            xa = x_ref[rs, :].astype(_F32) + mrow(2) * a
            xa_s[slot, rs, :] = xa
            hb = _ln(xa) * (1.0 + mrow(4)) + mrow(3)
            hb_s[slot, rs, :] = hb
            return _ln(hb).astype(_BF16)

        def mix_in(u, n):
            h1 = _gelu(_dot(n, w1[...]))
            h1_s[pl.ds(pl.multiple_of(PAD + i * T + u * R, 8), R), :] = h1

        h0 = ln1(0)
        h1_ = ln1(1)
        q0 = qkv(0, h0)

        @pl.when(i == 0)
        def _():
            cp_o.wait()
            for ct in range(G):
                cs = slice(ct * 128, (ct + 1) * 128)
                w32 = pltpu.bitcast(wo[:, cs], jnp.int32)
                for g in range(G):
                    pieces = []
                    for l in range(H):
                        hh = (l & 7) * 4 + (l >> 3)
                        r0 = hh * (Dh // 2) + g * 2
                        pieces.append(w32[r0:r0 + 2])
                    wo[g * 128:(g + 1) * 128, cs] = pltpu.bitcast(jnp.concatenate(pieces, axis=0), _BF16)
            mod_chunk(1)
            cp_1.wait()

        o0 = attn(0, q0)
        q1 = qkv(1, h1_)
        o1 = attn(1, q1)
        a0 = _dot(o0, wo[...])
        k_s[:, 0:HALO, :] = k_s[:, T:T + HALO, :]
        v_s[:, 0:HALO, :] = v_s[:, T:T + HALO, :]
        n0 = ln23(0, a0)
        a1 = _dot(o1, wo[...])
        n1 = ln23(1, a1)
        mix_in(0, n0)
        mix_in(1, n1)

    @pl.when(i == LAG)
    def _():
        mod_chunk(2)
        cp_2.wait()
        cp_3.wait()
        cp_4.wait()

    @pl.when(i >= LAG)
    def _():
        j = i - LAG
        slot = j % (LAG + 1)
        c4 = D // 4
        x1s, ns = [], []
        for u in range(NH):
            win = h1_s[pl.ds(pl.multiple_of(j * T + u * R, 8), R + 2 * PAD), :]
            g0 = win[PAD - 1:PAD - 1 + R, 0:c4]
            g1 = win[PAD + 1:PAD + 1 + R, c4:2 * c4]
            g2 = win[PAD - 2:PAD - 2 + R, 2 * c4:3 * c4]
            g3 = win[PAD + 2:PAD + 2 + R, 3 * c4:]
            gs = jnp.concatenate([g0, g1, g2, g3], axis=-1).astype(_BF16)
            x1 = hb_s[slot, u * R:(u + 1) * R, :] + _dot(gs, w2[...])
            x1s.append(x1)
            ns.append(_ln(x1).astype(_BF16))
        x1 = jnp.concatenate(x1s, axis=0)
        n1 = jnp.concatenate(ns, axis=0)
        h2 = None
        FC = 512
        for f in range(F // FC):
            w3f = w3[:, f * FC:(f + 1) * FC]
            if f == 0:
                t = jnp.concatenate([_dot(n, w3f) for n in ns], axis=0)
            else:
                t = _dot(n1, w3f)
            t = _dot(_gelu(t).astype(_BF16), w4[f * FC:(f + 1) * FC, :])
            h2 = t if h2 is None else h2 + t
        o_ref[...] = (xa_s[slot] + mrow(5) * (x1 + h2)).astype(o_ref.dtype)


@jax.jit
def pallas_adaLN_cond__sliding_local_dilated__mixer_s_mlp__prompt_kernel(
    A_x: jax.Array,
    A_wqkv: jax.Array,
    A_wo: jax.Array,
    B_x: jax.Array,
    B_w1: jax.Array,
    B_w2: jax.Array,
    B_w3: jax.Array,
    B_w4: jax.Array,
    c: jax.Array,
    w_mod: jax.Array,
):
    del B_x
    B, S, D = A_x.shape
    F = B_w3.shape[1]
    assert B == 1 and S % T == 0
    nT = S // T
    x2 = A_x.reshape(S, D)
    hbm = pl.BlockSpec(memory_space=pl.ANY)
    out = pl.pallas_call(
        functools.partial(_kernel, S=S, D=D, F=F),
        grid=(nT + LAG,),
        in_specs=[
            pl.BlockSpec((T, D), lambda i: (jnp.minimum(i, nT - 1), 0)),
            pl.BlockSpec((1, D), lambda i: (0, 0)),
            hbm, hbm, hbm, hbm, hbm, hbm, hbm,
        ],
        out_specs=pl.BlockSpec((T, D), lambda i: (jnp.maximum(i - LAG, 0), 0)),
        out_shape=jax.ShapeDtypeStruct((S, D), A_x.dtype),
        scratch_shapes=[
            pltpu.VMEM((D, 3 * D), _BF16),
            pltpu.VMEM((D, D), _BF16),
            pltpu.VMEM((D, D), _BF16),
            pltpu.VMEM((D, D), _BF16),
            pltpu.VMEM((D, F), _BF16),
            pltpu.VMEM((F, D), _BF16),
            pltpu.VMEM((D, 6 * D), _BF16),
            pltpu.VMEM((16, 6 * D), _F32),
            pltpu.VMEM((D // 128, HALO + T, 128), _F32),
            pltpu.VMEM((D // 128, HALO + T, 128), _F32),
            pltpu.VMEM((LAG + 1, T, D), _F32),
            pltpu.VMEM((LAG + 1, T, D), _F32),
            pltpu.VMEM((S + 2 * PAD, D), _F32),
            pltpu.SemaphoreType.DMA((12,)),
        ],
        compiler_params=pltpu.CompilerParams(
            dimension_semantics=("arbitrary",),
            vmem_limit_bytes=100 * 1024 * 1024,
        ),
    )(x2, c, A_wqkv, A_wo, B_w1, B_w2, B_w3, B_w4, w_mod)
    return out.reshape(B, S, D)
```
